```python
import os as _os
_os.environ.setdefault("JAX_PLATFORMS", "cpu")
import jax
import jax.numpy as jnp

def _softmax(x, axis=-1):
    return jax.nn.softmax(x, axis=axis)
def _gelu(x):
    return jax.nn.gelu(x, approximate=True)
def _silu(x):
    return jax.nn.silu(x)
def _sigmoid(x):
    return jax.nn.sigmoid(x)
def _layernorm(x, axis=-1, eps=1e-5):
    m = jnp.mean(x, axis=axis, keepdims=True)
    v = jnp.var(x, axis=axis, keepdims=True)
    return (x - m) / jnp.sqrt(v + eps)
def _scatter_add(tgt, idx, src, axis=0):
    return tgt.at[idx].add(src)
def _segment_sum(src, seg, n):
    return jax.ops.segment_sum(src, seg, n)
class _Rng:
    def __init__(self, key):
        self._k = key
    def _next(self):
        self._k, sub = jax.random.split(self._k)
        return sub
    def normal(self, shape):
        return jax.random.normal(self._next(), shape, dtype=jnp.bfloat16)
    def randint(self, lo, hi, shape):
        return jax.random.randint(self._next(), shape, lo, hi, dtype=jnp.int32)
    def uniform(self, shape, lo=0.0, hi=1.0):
        return jax.random.uniform(self._next(), shape, jnp.bfloat16, lo, hi)
    def permutation(self, n):
        return jax.random.permutation(self._next(), n)


kernel_name = 'standalone__geglu_ffn__prompt'

def setup_inputs():
    _rng = _Rng(jax.random.key(int.from_bytes(__import__("os").urandom(4), "little")))
    _w = (lambda a: (lambda t: t.astype(jnp.bfloat16) if jnp.issubdtype(t.dtype, jnp.floating) else t)(jnp.asarray(a)))
    B, S, D, F = 1, 2048, 576, 4608
    return {
        "x": _w((lambda *s: _rng.normal(s) * 0.05)(B, S, D)),
        "w_gate": _w((lambda *s: _rng.normal(s) * 0.05)(D, F)),
        "w_up": _w((lambda *s: _rng.normal(s) * 0.05)(D, F)),
        "w_down": _w((lambda *s: _rng.normal(s) * 0.05)(F, D)),
    }

def reference(x, w_gate, w_up, w_down):
    return (_gelu(x @ w_gate) * (x @ w_up)) @ w_down
```

```python
import jax
import jax.numpy as jnp
import jax.experimental.pallas as pl
import jax.experimental.pallas.tpu as pltpu


@jax.jit
def pallas_standalone__geglu_ffn__prompt_kernel(
    x: jax.Array,
    w_gate: jax.Array,
    w_up: jax.Array,
    w_down: jax.Array,
):
    B, S, D = x.shape
    F = w_gate.shape[1]
    M = B * S
    tm, tf = 1024, 1152

    def kernel(xT_ref, wg_ref, wu_ref, wdT_ref, oT_ref, x_scr, acc_ref):
        f = pl.program_id(1)

        @pl.when(f == 0)
        def _():
            x_scr[...] = xT_ref[...].T

        xb = x_scr[...]
        g = jnp.dot(xb, wg_ref[...], preferred_element_type=jnp.float32)
        u = jnp.dot(xb, wu_ref[...], preferred_element_type=jnp.float32)
        h = (jax.nn.gelu(g, approximate=True) * u).astype(jnp.bfloat16)
        p = jax.lax.dot_general(
            wdT_ref[...], h, (((1,), (1,)), ((), ())),
            preferred_element_type=jnp.float32)

        @pl.when(f == 0)
        def _():
            acc_ref[...] = p

        @pl.when(f > 0)
        def _():
            acc_ref[...] += p

        @pl.when(f == pl.num_programs(1) - 1)
        def _():
            oT_ref[...] = acc_ref[...].astype(oT_ref.dtype)

    xT = x.reshape(M, D).T
    wdT = w_down.T
    outT = pl.pallas_call(
        kernel,
        grid=(M // tm, F // tf),
        in_specs=[
            pl.BlockSpec((D, tm), lambda m, f: (0, m)),
            pl.BlockSpec((D, tf), lambda m, f: (0, f)),
            pl.BlockSpec((D, tf), lambda m, f: (0, f)),
            pl.BlockSpec((D, tf), lambda m, f: (0, f)),
        ],
        out_specs=pl.BlockSpec((D, tm), lambda m, f: (0, m)),
        out_shape=jax.ShapeDtypeStruct((D, M), x.dtype),
        scratch_shapes=[
            pltpu.VMEM((tm, D), jnp.bfloat16),
            pltpu.VMEM((D, tm), jnp.float32),
        ],
        compiler_params=pltpu.CompilerParams(
            dimension_semantics=("parallel", "arbitrary"),
            vmem_limit_bytes=100 * 1024 * 1024),
    )(xT, w_gate, w_up, wdT)
    return outT.T.reshape(B, S, D)
```

```python
import jax
import jax.numpy as jnp
from jax import lax
import jax.experimental.pallas as pl
import jax.experimental.pallas.tpu as pltpu

_NT = (((1,), (1,)), ((), ()))
_F32 = jnp.float32
_BF16 = jnp.bfloat16


def _act(g, u):
    return (jax.nn.gelu(g, approximate=True) * u).astype(_BF16)


def _mm(a, b):
    return jnp.dot(a, b, preferred_element_type=_F32)


def _mm_nt(a, b):
    return lax.dot_general(a, b, _NT, preferred_element_type=_F32)


@jax.jit
def pallas_standalone__geglu_ffn__prompt_kernel(
    x: jax.Array,
    w_gate: jax.Array,
    w_up: jax.Array,
    w_down: jax.Array,
):
    B, S, D = x.shape
    F = w_gate.shape[1]
    M = B * S
    assert (M, D, F) == (2048, 576, 4608)

    R1 = 256
    A = 256
    WC = 512
    TM = 1024
    TC = 2048
    G = 128
    NG = TM // G

    def kernel(xT_hbm, wg_hbm, wu_hbm, wdT_hbm, oT_hbm,
               xT_v, x_v, wg_v, wu_v, wd_v, acc, o_v, sem):
        w_h = (wg_hbm, wu_hbm, wdT_hbm)
        w_v = (wg_v, wu_v, wd_v)

        def wcopy(k, c0, n, s):
            sl = pl.ds(c0, n)
            return pltpu.make_async_copy(
                w_h[k].at[:, sl], w_v[k].at[:, sl], sem.at[s])

        def xcopy(r0, n, s):
            sl = pl.ds(r0, n)
            return pltpu.make_async_copy(
                xT_hbm.at[:, sl], xT_v.at[:, sl], sem.at[s])

        def ocopy(c0):
            sl = pl.ds(c0, G)
            return pltpu.make_async_copy(
                o_v.at[:, sl], oT_hbm.at[:, sl], sem.at[2])

        def transpose_x(r0, n):
            x_v[pl.ds(r0, n), :] = xT_v[:, pl.ds(r0, n)].T

        g0 = [xcopy(0, R1, 0)]
        g1 = [wcopy(0, 0, A, 1)]
        g2 = [wcopy(1, 0, A, 2), xcopy(R1, 512 - R1, 2)]
        g3 = [wcopy(2, 0, A, 3), xcopy(512, 512, 3)]
        g4 = [wcopy(k, A, WC - A, 4) for k in range(3)] + [xcopy(TM, TM, 4)]
        gc1 = [wcopy(k, WC, TC, 0) for k in range(3)]
        gc2 = [wcopy(k, WC + TC, TC, 1) for k in range(3)]

        for c in g0 + g1 + g2 + g3 + g4:
            c.start()

        s_a = pl.ds(0, A)
        halves = [(0, R1 // 2), (R1 // 2, R1 // 2)]

        for c in g0:
            c.wait()
        for c in gc1:
            c.start()
        transpose_x(0, R1)
        for c in g1:
            c.wait()
        for c in gc2:
            c.start()
        ga = [_mm(x_v[pl.ds(r, n), :], wg_v[:, s_a]) for r, n in halves]

        for c in g2:
            c.wait()
        transpose_x(R1, 512 - R1)
        ha = [_act(g_, _mm(x_v[pl.ds(r, n), :], wu_v[:, s_a]))
              for g_, (r, n) in zip(ga, halves)]
        xb = x_v[pl.ds(R1, 512 - R1), :]
        hb = _act(_mm(xb, wg_v[:, s_a]), _mm(xb, wu_v[:, s_a]))
        h0 = jnp.concatenate(ha + [hb], axis=0)

        for c in g3:
            c.wait()
        transpose_x(512, 512)
        acc[:, pl.ds(0, 512)] = _mm_nt(wd_v[:, s_a], h0)
        xb = x_v[pl.ds(512, 512), :]
        h1 = _act(_mm(xb, wg_v[:, s_a]), _mm(xb, wu_v[:, s_a]))
        acc[:, pl.ds(512, 512)] = _mm_nt(wd_v[:, s_a], h1)
        for c in g4:
            c.wait()

        def vbody(i, carry):
            first = i == 0
            r0 = pl.multiple_of(jnp.where(first, 0, TM), TM)
            rn = pl.multiple_of(jnp.where(first, TM, 0), TM)
            c0 = pl.multiple_of(jnp.where(i == 1, 0, A), A)
            sl = pl.ds(c0, A)
            xb = x_v[pl.ds(r0, TM), :]
            xn = xT_v[:, pl.ds(rn, TM)].T
            h = _act(_mm(xb, wg_v[:, sl]), _mm(xb, wu_v[:, sl]))
            prev = jnp.where(i == 1, 0.0, acc[:, pl.ds(r0, TM)])
            acc[:, pl.ds(r0, TM)] = prev + _mm_nt(wd_v[:, sl], h)
            x_v[pl.ds(rn, TM), :] = xn
            return carry

        lax.fori_loop(0, 3, vbody, 0)
        for c in gc1:
            c.wait()

        def mbody(i, carry):
            @pl.when(i == 2)
            def _():
                for c in gc2:
                    c.wait()

            r0 = pl.multiple_of((i % 2) * TM, TM)
            c0 = pl.multiple_of(WC + (i // 2) * TC, 128)
            sl = pl.ds(c0, TC)
            xb = x_v[pl.ds(r0, TM), :]
            h = _act(_mm(xb, wg_v[:, sl]), _mm(xb, wu_v[:, sl]))
            wd = wd_v[:, sl]
            for g_ in range(NG):
                osl = pl.ds(pl.multiple_of(r0 + g_ * G, 128), G)
                val = acc[:, osl] + _mm_nt(wd, h[g_ * G:(g_ + 1) * G])
                acc[:, osl] = val
                o_v[:, osl] = val.astype(o_v.dtype)

                @pl.when(i == 2)
                def _():
                    ocopy(g_ * G).start()

                @pl.when(i == 3)
                def _():
                    ocopy(TM + g_ * G).start()
            return carry

        lax.fori_loop(0, 4, mbody, 0)
        pltpu.make_async_copy(o_v, oT_hbm, sem.at[2]).wait()

    any_spec = pl.BlockSpec(memory_space=pl.ANY)
    out_t = pl.pallas_call(
        kernel,
        in_specs=[any_spec] * 4,
        out_specs=any_spec,
        out_shape=jax.ShapeDtypeStruct((D, M), x.dtype),
        scratch_shapes=[
            pltpu.VMEM((D, M), _BF16),
            pltpu.VMEM((M, D), _BF16),
            pltpu.VMEM((D, F), _BF16),
            pltpu.VMEM((D, F), _BF16),
            pltpu.VMEM((D, F), _BF16),
            pltpu.VMEM((D, M), _F32),
            pltpu.VMEM((D, M), _BF16),
            pltpu.SemaphoreType.DMA((5,)),
        ],
        compiler_params=pltpu.CompilerParams(
            vmem_limit_bytes=110 * 1024 * 1024),
    )(x.reshape(M, D).T, w_gate, w_up, w_down.T)
    return out_t.T.reshape(B, S, D)
```

```python
import math

import jax
import jax.numpy as jnp
from jax import lax
import jax.experimental.pallas as pl
import jax.experimental.pallas.tpu as pltpu

_NT = (((1,), (1,)), ((), ()))
_F32 = jnp.float32
_BF16 = jnp.bfloat16
_C1 = math.sqrt(2.0 / math.pi)
_C2 = _C1 * 0.044715


def _act2(g, u):
    t = jnp.tanh(g * (_C1 + _C2 * (g * g)))
    return (g * u) * (1.0 + t)


def _mm(a, b):
    return jnp.dot(a, b, preferred_element_type=_F32)


def _mm_nt(a, b):
    return lax.dot_general(a, b, _NT, preferred_element_type=_F32)


@jax.jit
def pallas_standalone__geglu_ffn__prompt_kernel(
    x: jax.Array,
    w_gate: jax.Array,
    w_up: jax.Array,
    w_down: jax.Array,
):
    B, S, D = x.shape
    F = w_gate.shape[1]
    M = B * S
    assert (M, D, F) == (2048, 576, 4608)

    A = 256
    Q = 512
    TC = 1024
    NP = 4
    WP = 1280
    G = 128
    LAST = (288, 144, 96, 32, 16)
    assert 2 * A + NP * TC == F and 4 * Q == M and sum(LAST) == D

    def kernel(xT_hbm, wg_hbm, wu_hbm, wdT_hbm, oT_hbm,
               xT_v, x_v, wgs, wus, wds, wgm, wum, wdm, acc, o_v, sem):
        w_hbm = (wg_hbm, wu_hbm, wdT_hbm)
        w_small = (wgs, wus, wds)
        w_main = (wgm, wum, wdm)

        def small_copy(k, j, s):
            return pltpu.make_async_copy(
                w_hbm[k].at[:, pl.ds(j * A, A)], w_small[k].at[j], sem.at[s])

        def main_copy(k, p, s):
            return pltpu.make_async_copy(
                w_hbm[k].at[:, pl.ds(2 * A + p * TC, TC)],
                w_main[k].at[p, :, pl.ds(0, TC)], sem.at[s])

        def x_copy(r0, n, s):
            return pltpu.make_async_copy(
                xT_hbm.at[:, pl.ds(r0, n)], xT_v.at[:, pl.ds(r0, n)],
                sem.at[s])

        def out_copy(c0, d0, nd):
            return pltpu.make_async_copy(
                o_v.at[pl.ds(d0, nd), pl.ds(c0, G)],
                oT_hbm.at[pl.ds(d0, nd), pl.ds(c0, G)], sem.at[2])

        def transpose_x(r0, n):
            q, r = divmod(r0, Q)
            x_v[q, pl.ds(r, n), :] = xT_v[:, pl.ds(r0, n)].T

        def rows(q, r=0, n=Q):
            return x_v[q, pl.ds(r, n), :]

        def gate_up(xb, j):
            return _act2(_mm(xb, wgs[j]), _mm(xb, wus[j])).astype(_BF16)

        def start(group):
            for c in group:
                c.start()

        def wait(group):
            for c in group:
                c.wait()

        g0 = [x_copy(0, 256, 0)]
        g1 = [small_copy(0, 0, 1)]
        g2a = [small_copy(1, 0, 5)]
        g2 = [x_copy(256, 256, 2)]
        g3 = [small_copy(2, 0, 3), x_copy(512, 256, 3)]
        g4 = [x_copy(768, M - 768, 4)]
        gc0 = ([small_copy(k, 1, 0) for k in range(3)]
               + [main_copy(k, 0, 0) for k in range(3)])
        gcr = [main_copy(k, p, 1) for p in range(1, NP) for k in range(3)]

        start(g0 + g1 + g2a + g2 + g3 + g4)

        wait(g0)
        start(gc0)
        transpose_x(0, 256)
        wait(g1)
        start(gcr)
        ga = [_mm(rows(0, r, 128), wgs[0]) for r in (0, 128)]

        def up_act(r):
            g = ga[r // 128][r % 128:r % 128 + 64]
            return _act2(g, _mm(rows(0, r, 64), wus[0])).astype(_BF16)

        wait(g2a)
        h0 = [up_act(0), up_act(64)]
        wait(g2)
        transpose_x(256, 256)
        h0 += [up_act(128), up_act(192), gate_up(rows(0, 256, 256), 0)]
        h0 = jnp.concatenate(h0, axis=0)

        wait(g3)
        transpose_x(512, 256)
        acc[0] = _mm_nt(wds[0], h0)
        h1a = gate_up(rows(1, 0, 256), 0)

        wait(g4)
        transpose_x(768, 256)
        acc[1, :, pl.ds(0, 256)] = _mm_nt(wds[0], h1a)
        transpose_x(1024, Q)
        h1b = gate_up(rows(1, 256, 256), 0)
        transpose_x(1536, Q)
        h2 = gate_up(rows(2), 0)
        acc[1, :, pl.ds(256, 256)] = _mm_nt(wds[0], h1b)
        h3 = gate_up(rows(3), 0)
        acc[2] = _mm_nt(wds[0], h2)
        acc[3] = _mm_nt(wds[0], h3)
        wait(gc0)

        def body(i, carry):
            @pl.when(i == 1)
            def _():
                wait(gcr)

            cols = pl.ds(0, TC)
            xb = x_v[...].reshape(M, D)
            hf = _act2(_mm(xb, wgm[i, :, cols]), _mm(xb, wum[i, :, cols]))
            wd = wdm[i, :, cols]
            for q in range(4):
                if q == 3:
                    acc[i] += _mm_nt(wds[1], gate_up(rows(i), 1))
                for g in range(Q // G):
                    c0 = q * Q + g * G
                    osl = pl.ds(g * G, G)
                    val = acc[q, :, osl] + _mm_nt(
                        wd, hf[c0:c0 + G].astype(_BF16))
                    acc[q, :, osl] = val
                    d0 = 0
                    for nd in (LAST if c0 + G == M else (D,)):
                        o_v[pl.ds(d0, nd), pl.ds(c0, G)] = (
                            val[d0:d0 + nd] * 0.5).astype(o_v.dtype)

                        @pl.when(i == NP - 1)
                        def _():
                            out_copy(c0, d0, nd).start()

                        d0 += nd
            return carry

        lax.fori_loop(0, NP, body, 0)
        pltpu.make_async_copy(o_v, o_v, sem.at[2]).wait()

    any_spec = pl.BlockSpec(memory_space=pl.ANY)
    out_t = pl.pallas_call(
        kernel,
        in_specs=[any_spec] * 4,
        out_specs=any_spec,
        out_shape=jax.ShapeDtypeStruct((D, M), x.dtype),
        scratch_shapes=[
            pltpu.VMEM((D, M), _BF16),
            pltpu.VMEM((4, Q, D), _BF16),
            pltpu.VMEM((2, D, A), _BF16),
            pltpu.VMEM((2, D, A), _BF16),
            pltpu.VMEM((2, D, A), _BF16),
            pltpu.VMEM((NP, D, WP), _BF16),
            pltpu.VMEM((NP, D, WP), _BF16),
            pltpu.VMEM((NP, D, WP), _BF16),
            pltpu.VMEM((4, D, Q), _F32),
            pltpu.VMEM((D, M), _BF16),
            pltpu.SemaphoreType.DMA((6,)),
        ],
        compiler_params=pltpu.CompilerParams(
            vmem_limit_bytes=110 * 1024 * 1024),
    )(x.reshape(M, D).T, w_gate, w_up, w_down.T)
    return out_t.T.reshape(B, S, D)
```

```python
import math

import jax
import jax.numpy as jnp
from jax import lax
import jax.experimental.pallas as pl
import jax.experimental.pallas.tpu as pltpu

_NT = (((1,), (1,)), ((), ()))
_F32 = jnp.float32
_BF16 = jnp.bfloat16
_C1 = math.sqrt(2.0 / math.pi)
_C2 = _C1 * 0.044715


def _act2(g, u):
    t = jnp.tanh(g * (_C1 + _C2 * (g * g)))
    return (g * (1.0 + t)) * u


def _mm(a, b):
    return jnp.dot(a, b, preferred_element_type=_F32)


def _mm_nt(a, b):
    return lax.dot_general(a, b, _NT, preferred_element_type=_F32)


@jax.jit
def pallas_standalone__geglu_ffn__prompt_kernel(
    x: jax.Array,
    w_gate: jax.Array,
    w_up: jax.Array,
    w_down: jax.Array,
):
    B, S, D = x.shape
    F = w_gate.shape[1]
    M = B * S
    assert (M, D, F) == (2048, 576, 4608)

    A = 256
    Q = 512
    TC = 1024
    NP = 4
    WP = 1280
    G = 128
    LAST = (288, 144, 96, 32, 16)
    assert 2 * A + NP * TC == F and 4 * Q == M and sum(LAST) == D

    def kernel(xT_hbm, wg_hbm, wu_hbm, wdT_hbm, oT_hbm,
               xT_v, x_v, wgs, wus, wds, wgm, wum, wdm, acc, o_v, sem):
        w_hbm = (wg_hbm, wu_hbm, wdT_hbm)
        w_small = (wgs, wus, wds)
        w_main = (wgm, wum, wdm)

        def small_copy(k, j, s):
            return pltpu.make_async_copy(
                w_hbm[k].at[:, pl.ds(j * A, A)], w_small[k].at[j], sem.at[s])

        def main_copy(k, p, s):
            return pltpu.make_async_copy(
                w_hbm[k].at[:, pl.ds(2 * A + p * TC, TC)],
                w_main[k].at[p, :, pl.ds(0, TC)], sem.at[s])

        def x_copy(r0, n, s):
            return pltpu.make_async_copy(
                xT_hbm.at[:, pl.ds(r0, n)], xT_v.at[:, pl.ds(r0, n)],
                sem.at[s])

        def out_copy(c0, d0, nd):
            return pltpu.make_async_copy(
                o_v.at[pl.ds(d0, nd), pl.ds(c0, G)],
                oT_hbm.at[pl.ds(d0, nd), pl.ds(c0, G)], sem.at[2])

        def transpose_x(r0, n):
            q, r = divmod(r0, Q)
            x_v[q, pl.ds(r, n), :] = xT_v[:, pl.ds(r0, n)].T

        def rows(q, r=0, n=Q):
            return x_v[q, pl.ds(r, n), :]

        def gate_up(xb, j):
            return _act2(_mm(xb, wgs[j]), _mm(xb, wus[j])).astype(_BF16)

        def start(group):
            for c in group:
                c.start()

        def wait(group):
            for c in group:
                c.wait()

        g0 = [x_copy(0, 256, 0)]
        g1 = [small_copy(0, 0, 1)]
        g2a = [small_copy(1, 0, 5)]
        g2 = [x_copy(256, 256, 2)]
        g3 = [small_copy(2, 0, 3), x_copy(512, 384, 3)]
        g4 = [x_copy(896, M - 896, 4)]
        gc0 = ([small_copy(k, 1, 0) for k in range(3)]
               + [main_copy(k, 0, 0) for k in range(3)])
        gcr = [main_copy(k, p, 1) for p in range(1, NP) for k in range(3)]

        start(g0 + g1 + g2a + g2 + g3 + g4)

        def warmup():
            wait(g0)
            start(gc0)
            transpose_x(0, 256)
            wait(g1)
            start(gcr)
            ga = [_mm(rows(0, r, 128), wgs[0]) for r in (0, 128)]

            def up_act(r):
                g = ga[r // 128][r % 128:r % 128 + 64]
                return _act2(g, _mm(rows(0, r, 64), wus[0])).astype(_BF16)

            wait(g2a)
            h0 = [up_act(0), up_act(64)]
            wait(g2)
            transpose_x(256, 256)
            h0 += [up_act(128), up_act(192), gate_up(rows(0, 256, 256), 0)]
            h0 = jnp.concatenate(h0, axis=0)

            wait(g3)
            transpose_x(512, 384)
            acc[0] = _mm_nt(wds[0], h0)
            h1a = gate_up(rows(1, 0, 384), 0)

            wait(g4)
            transpose_x(896, 128)
            acc[1, :, pl.ds(0, 256)] = _mm_nt(wds[0], h1a[:256])
            transpose_x(1024, Q)
            h1b = jnp.concatenate(
                [h1a[256:], gate_up(rows(1, 384, 128), 0)], axis=0)
            transpose_x(1536, Q)
            h2 = gate_up(rows(2), 0)
            acc[1, :, pl.ds(256, 256)] = _mm_nt(wds[0], h1b)
            h3 = gate_up(rows(3), 0)
            acc[2] = _mm_nt(wds[0], h2)
            acc[3] = _mm_nt(wds[0], h3)
            wait(gc0)

        def body(i, carry):
            pl.when(i == 0)(warmup)

            @pl.when(i == 1)
            def _():
                wait(gcr)

            cols = pl.ds(0, TC)
            xb = x_v[...].reshape(M, D)
            hf = _act2(_mm(xb, wgm[i, :, cols]), _mm(xb, wum[i, :, cols]))
            wd = wdm[i, :, cols]
            for q in range(4):
                if q == 3:
                    acc[i] += _mm_nt(wds[1], gate_up(rows(i), 1))
                for g in range(Q // G):
                    c0 = q * Q + g * G
                    osl = pl.ds(g * G, G)
                    val = acc[q, :, osl] + _mm_nt(
                        wd, hf[c0:c0 + G].astype(_BF16))
                    acc[q, :, osl] = val
                    d0 = 0
                    for nd in (LAST if c0 + G == M else (D,)):
                        o_v[pl.ds(d0, nd), pl.ds(c0, G)] = (
                            val[d0:d0 + nd] * 0.5).astype(o_v.dtype)

                        @pl.when(i == NP - 1)
                        def _():
                            out_copy(c0, d0, nd).start()

                        d0 += nd
            return carry

        lax.fori_loop(0, NP, body, 0)
        pltpu.make_async_copy(o_v, o_v, sem.at[2]).wait()

    any_spec = pl.BlockSpec(memory_space=pl.ANY)
    out_t = pl.pallas_call(
        kernel,
        in_specs=[any_spec] * 4,
        out_specs=any_spec,
        out_shape=jax.ShapeDtypeStruct((D, M), x.dtype),
        scratch_shapes=[
            pltpu.VMEM((D, M), _BF16),
            pltpu.VMEM((4, Q, D), _BF16),
            pltpu.VMEM((2, D, A), _BF16),
            pltpu.VMEM((2, D, A), _BF16),
            pltpu.VMEM((2, D, A), _BF16),
            pltpu.VMEM((NP, D, WP), _BF16),
            pltpu.VMEM((NP, D, WP), _BF16),
            pltpu.VMEM((NP, D, WP), _BF16),
            pltpu.VMEM((4, D, Q), _F32),
            pltpu.VMEM((D, M), _BF16),
            pltpu.SemaphoreType.DMA((6,)),
        ],
        compiler_params=pltpu.CompilerParams(
            vmem_limit_bytes=110 * 1024 * 1024),
    )(x.reshape(M, D).T, w_gate, w_up, w_down.T)
    return out_t.T.reshape(B, S, D)
```

```python
import math

import jax
import jax.numpy as jnp
from jax import lax
import jax.experimental.pallas as pl
import jax.experimental.pallas.tpu as pltpu

_NT = (((1,), (1,)), ((), ()))
_F32 = jnp.float32
_BF16 = jnp.bfloat16
_C1 = math.sqrt(2.0 / math.pi)
_C2 = _C1 * 0.044715


def _act2(g, u):
    t = jnp.tanh(g * (_C1 + _C2 * (g * g)))
    return (g * (1.0 + t)) * u


def _mm(a, b):
    return jnp.dot(a, b, preferred_element_type=_F32)


def _mm_nt(a, b):
    return lax.dot_general(a, b, _NT, preferred_element_type=_F32)


@jax.jit
def pallas_standalone__geglu_ffn__prompt_kernel(
    x: jax.Array,
    w_gate: jax.Array,
    w_up: jax.Array,
    w_down: jax.Array,
):
    B, S, D = x.shape
    F = w_gate.shape[1]
    M = B * S
    assert (M, D, F) == (2048, 576, 4608)

    A = 256
    Q = 512
    TC = 1024
    NP = 4
    WP = 1280
    G = 128
    LAST = (288, 144, 96, 32, 16)
    KT = 128
    KR = 3 * KT
    assert 2 * A + NP * TC == F and 4 * Q == M and sum(LAST) == D

    STAGES = (
        ((), ((0, 0, 1),)),
        ((), ((0, 1, 2),)),
        ((1,), ((0, 3, 1), (1, 0, 2))),
        ((2,), ((1, 2, 2), (2, 0, 3))),
    )

    def kernel(xT_hbm, wg_hbm, wu_hbm, wdT_hbm, oT_hbm,
               xT_v, x_v, wgs, wus, wds, wgm, wum, wdm, acc, o_v, wT, gu, sem):
        w_hbm = (wg_hbm, wu_hbm, wdT_hbm)
        w_small = (wgs, wus, wds)
        w_main = (wgm, wum, wdm)

        def small_copy(k, j, s):
            return pltpu.make_async_copy(
                w_hbm[k].at[:, pl.ds(j * A, A)], w_small[k].at[j], sem.at[s])

        def main_copy(k, p, s):
            return pltpu.make_async_copy(
                w_hbm[k].at[:, pl.ds(2 * A + p * TC, TC)],
                w_main[k].at[p, :, pl.ds(0, TC)], sem.at[s])

        def x_slab_copy(k0, nk, t0, n, s):
            return pltpu.make_async_copy(
                xT_hbm.at[pl.ds(k0, nk), pl.ds(t0, n)],
                xT_v.at[pl.ds(k0, nk), pl.ds(t0, n)], sem.at[s])

        def w_slab_copies(k0, nk, s):
            return [pltpu.make_async_copy(
                w_hbm[k].at[pl.ds(k0, nk), pl.ds(0, A)],
                w_small[k].at[0, pl.ds(k0, nk), :], sem.at[s])
                for k in range(2)]

        def out_copy(c0, d0, nd):
            return pltpu.make_async_copy(
                o_v.at[pl.ds(d0, nd), pl.ds(c0, G)],
                oT_hbm.at[pl.ds(d0, nd), pl.ds(c0, G)], sem.at[2])

        def start(group):
            for c in group:
                c.start()

        def wait(group):
            for c in group:
                c.wait()

        g_w0 = w_slab_copies(0, KT, 0)
        g_stage = []
        for si, (slabs, parts) in enumerate(STAGES):
            g = [c for k in slabs for c in w_slab_copies(k * KT, KT, si + 1)]
            g += [x_slab_copy(k * KT, KT, q0 * Q, nq * Q, si + 1)
                  for k, q0, nq in parts]
            g_stage.append(g)
        g_last = ([x_slab_copy(2 * KT, KT, 3 * Q, Q, 5)]
                  + w_slab_copies(KR, D - KR, 5)
                  + [x_slab_copy(KR, D - KR, 0, M, 5), small_copy(2, 0, 5)])
        g_main0 = ([small_copy(k, 1, 0) for k in range(3)]
                   + [main_copy(k, 0, 0) for k in range(3)])
        g_rest = [main_copy(k, p, 1) for p in range(1, NP) for k in range(3)]

        start(g_w0 + [c for g in g_stage for c in g] + g_last)

        def transpose_w(k0, nk):
            wT[pl.ds(0, A), pl.ds(k0, nk)] = wgs[0, pl.ds(k0, nk), :].T
            wT[pl.ds(A, A), pl.ds(k0, nk)] = wus[0, pl.ds(k0, nk), :].T

        def gate_up_t(k0, nk, q):
            return _mm(wT[:, pl.ds(k0, nk)],
                       xT_v[pl.ds(k0, nk), pl.ds(q * Q, Q)])

        def accumulate(k, q):
            if k == 0:
                gu[q] = gate_up_t(0, KT, q)
            else:
                gu[q] += gate_up_t(k * KT, KT, q)

        def warmup():
            wait(g_w0)
            start(g_main0)
            transpose_w(0, KT)
            for si, (slabs, parts) in enumerate(STAGES):
                wait(g_stage[si])
                if si == 0:
                    start(g_rest)
                for k in slabs:
                    transpose_w(k * KT, KT)
                for k, q0, nq in parts:
                    for q in range(q0, q0 + nq):
                        accumulate(k, q)
            wait(g_last)
            transpose_w(KR, D - KR)
            accumulate(2, 3)
            h_t = []
            for q in range(4):
                v = gu[q] + gate_up_t(KR, D - KR, q)
                h_t.append(_act2(v[:A], v[A:]).astype(_BF16))
            for q in range(4):
                acc[q] = _mm(wds[0], h_t[q])
                x_v[q] = xT_v[:, pl.ds(q * Q, Q)].T
            wait(g_main0)

        def body(i, carry):
            pl.when(i == 0)(warmup)

            @pl.when(i == 1)
            def _():
                wait(g_rest)

            cols = pl.ds(0, TC)
            xb = x_v[...].reshape(M, D)
            hf = _act2(_mm(xb, wgm[i, :, cols]), _mm(xb, wum[i, :, cols]))
            wd = wdm[i, :, cols]
            for q in range(4):
                if q == 3:
                    xe = x_v[i]
                    he = _act2(_mm(xe, wgs[1]), _mm(xe, wus[1]))
                    acc[i] += _mm_nt(wds[1], he.astype(_BF16))
                for g in range(Q // G):
                    c0 = q * Q + g * G
                    osl = pl.ds(g * G, G)
                    val = acc[q, :, osl] + _mm_nt(
                        wd, hf[c0:c0 + G].astype(_BF16))
                    acc[q, :, osl] = val
                    d0 = 0
                    for nd in (LAST if c0 + G == M else (D,)):
                        o_v[pl.ds(d0, nd), pl.ds(c0, G)] = (
                            val[d0:d0 + nd] * 0.5).astype(o_v.dtype)

                        @pl.when(i == NP - 1)
                        def _():
                            out_copy(c0, d0, nd).start()

                        d0 += nd
            return carry

        lax.fori_loop(0, NP, body, 0)
        pltpu.make_async_copy(o_v, o_v, sem.at[2]).wait()

    any_spec = pl.BlockSpec(memory_space=pl.ANY)
    out_t = pl.pallas_call(
        kernel,
        in_specs=[any_spec] * 4,
        out_specs=any_spec,
        out_shape=jax.ShapeDtypeStruct((D, M), x.dtype),
        scratch_shapes=[
            pltpu.VMEM((D, M), _BF16),
            pltpu.VMEM((4, Q, D), _BF16),
            pltpu.VMEM((2, D, A), _BF16),
            pltpu.VMEM((2, D, A), _BF16),
            pltpu.VMEM((2, D, A), _BF16),
            pltpu.VMEM((NP, D, WP), _BF16),
            pltpu.VMEM((NP, D, WP), _BF16),
            pltpu.VMEM((NP, D, WP), _BF16),
            pltpu.VMEM((4, D, Q), _F32),
            pltpu.VMEM((D, M), _BF16),
            pltpu.VMEM((2 * A, D), _BF16),
            pltpu.VMEM((4, 2 * A, Q), _F32),
            pltpu.SemaphoreType.DMA((6,)),
        ],
        compiler_params=pltpu.CompilerParams(
            vmem_limit_bytes=110 * 1024 * 1024),
    )(x.reshape(M, D).T, w_gate, w_up, w_down.T)
    return out_t.T.reshape(B, S, D)
```

```python
import math

import jax
import jax.numpy as jnp
from jax import lax
import jax.experimental.pallas as pl
import jax.experimental.pallas.tpu as pltpu

_NT = (((1,), (1,)), ((), ()))
_F32 = jnp.float32
_BF16 = jnp.bfloat16
_C1 = math.sqrt(2.0 / math.pi)
_C2 = _C1 * 0.044715


def _act2(g, u):
    t = jnp.tanh(g * (_C1 + _C2 * (g * g)))
    return (g * (1.0 + t)) * u


def _mm(a, b):
    return jnp.dot(a, b, preferred_element_type=_F32)


def _mm_nt(a, b):
    return lax.dot_general(a, b, _NT, preferred_element_type=_F32)


@jax.jit
def pallas_standalone__geglu_ffn__prompt_kernel(
    x: jax.Array,
    w_gate: jax.Array,
    w_up: jax.Array,
    w_down: jax.Array,
):
    B, S, D = x.shape
    F = w_gate.shape[1]
    M = B * S
    assert (M, D, F) == (2048, 576, 4608)

    A = 256
    Q = 512
    TC = 1024
    NP = 4
    WP = 1280
    G = 128
    LAST = (288, 144, 96, 32, 16)
    assert 2 * A + NP * TC == F and 4 * Q == M and sum(LAST) == D

    SLAB = ((512, 64), (0, 128), (128, 128), (256, 256))
    STAGES = (
        ((), ((0, 0, 3),)),
        ((1,), ((0, 3, 1), (1, 0, 3))),
        ((2, 3), ((1, 3, 1), (2, 0, 4))),
    )

    def kernel(xT_hbm, wg_hbm, wu_hbm, wdT_hbm, oT_hbm,
               xT_v, x_v, wgs, wus, wds, wgm, wum, wdm, acc, o_v, wT, gu, sem):
        w_hbm = (wg_hbm, wu_hbm, wdT_hbm)
        w_small = (wgs, wus, wds)
        w_main = (wgm, wum, wdm)

        def small_copy(k, j, s):
            return pltpu.make_async_copy(
                w_hbm[k].at[:, pl.ds(j * A, A)], w_small[k].at[j], sem.at[s])

        def main_copy(k, p, s):
            return pltpu.make_async_copy(
                w_hbm[k].at[:, pl.ds(2 * A + p * TC, TC)],
                w_main[k].at[p, :, pl.ds(0, TC)], sem.at[s])

        def x_slab_copy(k, q0, nq, s):
            idx = (pl.ds(*SLAB[k]), pl.ds(q0 * Q, nq * Q))
            return pltpu.make_async_copy(
                xT_hbm.at[idx], xT_v.at[idx], sem.at[s])

        def w_slab_copies(k, s):
            return [pltpu.make_async_copy(
                w_hbm[m].at[pl.ds(*SLAB[k]), pl.ds(0, A)],
                w_small[m].at[0, pl.ds(*SLAB[k]), :], sem.at[s])
                for m in range(2)]

        def out_copy(c0, d0, nd):
            return pltpu.make_async_copy(
                o_v.at[pl.ds(d0, nd), pl.ds(c0, G)],
                oT_hbm.at[pl.ds(d0, nd), pl.ds(c0, G)], sem.at[2])

        def start(group):
            for c in group:
                c.start()

        def wait(group):
            for c in group:
                c.wait()

        g_w0 = w_slab_copies(0, 0)
        g_stage = []
        for si, (slabs, parts) in enumerate(STAGES):
            now = [k for k in slabs if any(p[0] == k for p in parts)]
            ahead = [k for k in slabs if k not in now]
            g_stage.append(
                [c for k in now for c in w_slab_copies(k, si + 1)]
                + [x_slab_copy(k, q0, nq, si + 1) for k, q0, nq in parts]
                + [c for k in ahead for c in w_slab_copies(k, si + 1)])
        g_last = [x_slab_copy(3, 0, 4, 4), small_copy(2, 0, 4)]
        g_main0 = ([small_copy(k, 1, 0) for k in range(3)]
                   + [main_copy(k, 0, 0) for k in range(3)])
        g_rest = [main_copy(k, p, 1) for p in range(1, NP) for k in range(3)]

        start(g_w0 + [c for g in g_stage for c in g] + g_last)

        def transpose_w(k):
            ks = pl.ds(*SLAB[k])
            wT[pl.ds(0, A), ks] = wgs[0, ks, :].T
            wT[pl.ds(A, A), ks] = wus[0, ks, :].T

        def gate_up_t(k, q):
            ks = pl.ds(*SLAB[k])
            return _mm(wT[:, ks], xT_v[ks, pl.ds(q * Q, Q)])

        def warmup():
            wait(g_w0)
            start(g_main0)
            transpose_w(0)
            for si, (slabs, parts) in enumerate(STAGES):
                wait(g_stage[si])
                if si == 0:
                    start(g_rest)
                for k in slabs:
                    transpose_w(k)
                for k, q0, nq in parts:
                    for q in range(q0, q0 + nq):
                        if k == 0:
                            gu[q] = gate_up_t(k, q)
                        else:
                            gu[q] += gate_up_t(k, q)
            wait(g_last)
            h_t = []
            for q in range(4):
                v = gu[q] + gate_up_t(3, q)
                h_t.append(_act2(v[:A], v[A:]).astype(_BF16))
            for q in range(4):
                acc[q] = _mm(wds[0], h_t[q])
                x_v[q] = xT_v[:, pl.ds(q * Q, Q)].T
            wait(g_main0)

        def body(i, carry):
            pl.when(i == 0)(warmup)

            @pl.when(i == 1)
            def _():
                wait(g_rest)

            cols = pl.ds(0, TC)
            xb = x_v[...].reshape(M, D)
            hf = _act2(_mm(xb, wgm[i, :, cols]), _mm(xb, wum[i, :, cols]))
            wd = wdm[i, :, cols]
            for q in range(4):
                if q == 3:
                    xe = x_v[i]
                    he = _act2(_mm(xe, wgs[1]), _mm(xe, wus[1]))
                    acc[i] += _mm_nt(wds[1], he.astype(_BF16))
                for g in range(Q // G):
                    c0 = q * Q + g * G
                    osl = pl.ds(g * G, G)
                    val = acc[q, :, osl] + _mm_nt(
                        wd, hf[c0:c0 + G].astype(_BF16))
                    acc[q, :, osl] = val
                    d0 = 0
                    for nd in (LAST if c0 + G == M else (D,)):
                        o_v[pl.ds(d0, nd), pl.ds(c0, G)] = (
                            val[d0:d0 + nd] * 0.5).astype(o_v.dtype)

                        @pl.when(i == NP - 1)
                        def _():
                            out_copy(c0, d0, nd).start()

                        d0 += nd
            return carry

        lax.fori_loop(0, NP, body, 0)
        pltpu.make_async_copy(o_v, o_v, sem.at[2]).wait()

    any_spec = pl.BlockSpec(memory_space=pl.ANY)
    out_t = pl.pallas_call(
        kernel,
        in_specs=[any_spec] * 4,
        out_specs=any_spec,
        out_shape=jax.ShapeDtypeStruct((D, M), x.dtype),
        scratch_shapes=[
            pltpu.VMEM((D, M), _BF16),
            pltpu.VMEM((4, Q, D), _BF16),
            pltpu.VMEM((2, D, A), _BF16),
            pltpu.VMEM((2, D, A), _BF16),
            pltpu.VMEM((2, D, A), _BF16),
            pltpu.VMEM((NP, D, WP), _BF16),
            pltpu.VMEM((NP, D, WP), _BF16),
            pltpu.VMEM((NP, D, WP), _BF16),
            pltpu.VMEM((4, D, Q), _F32),
            pltpu.VMEM((D, M), _BF16),
            pltpu.VMEM((2 * A, D), _BF16),
            pltpu.VMEM((4, 2 * A, Q), _F32),
            pltpu.SemaphoreType.DMA((5,)),
        ],
        compiler_params=pltpu.CompilerParams(
            vmem_limit_bytes=110 * 1024 * 1024),
    )(x.reshape(M, D).T, w_gate, w_up, w_down.T)
    return out_t.T.reshape(B, S, D)
```

```python
import math

import jax
import jax.numpy as jnp
from jax import lax
import jax.experimental.pallas as pl
import jax.experimental.pallas.tpu as pltpu

_NT = (((1,), (1,)), ((), ()))
_F32 = jnp.float32
_BF16 = jnp.bfloat16
_C1 = math.sqrt(2.0 / math.pi)
_C2 = _C1 * 0.044715


def _act2(g, u):
    t = jnp.tanh(g * (_C1 + _C2 * (g * g)))
    return (g * (1.0 + t)) * u


def _mm(a, b):
    return jnp.dot(a, b, preferred_element_type=_F32)


def _mm_nt(a, b):
    return lax.dot_general(a, b, _NT, preferred_element_type=_F32)


@jax.jit
def pallas_standalone__geglu_ffn__prompt_kernel(
    x: jax.Array,
    w_gate: jax.Array,
    w_up: jax.Array,
    w_down: jax.Array,
):
    B, S, D = x.shape
    F = w_gate.shape[1]
    M = B * S
    assert (M, D, F) == (2048, 576, 4608)

    A = 384
    NE = 3
    TC = 640
    NP = 6
    CHUNKS = (256, 256, 128)
    Q, H = 512, 1024
    G = 128
    LAST = (288, 144, 96, 32, 16)
    KM, KR = 512, 64
    assert A + NE * 128 + NP * TC == F and sum(CHUNKS) == TC
    assert sum(LAST) == D and KM + KR == D and 2 * NE == NP

    SLAB = ((512, 64), (0, 128), (128, 128), (256, 256))
    STAGES = (
        ((), ((0, 0, 3),)),
        ((1, 2), ((0, 3, 1), (1, 0, 4), (2, 0, 1))),
    )
    LEFT = ((2, 1, 3),)

    GR = 16
    NGRP = M // GR
    V1 = [12 + 10 * j for j in range(12)]
    rest = [g for g in range(NGRP) if g not in V1]
    V2 = [rest[(2 * j + 1) * len(rest) // 16] for j in range(8)]
    VALL = V1 + V2
    NV, NV2 = GR * len(VALL), GR * len(V2)
    MV = M - NV
    RUNS, g = [], 0
    while g < NGRP:
        if g in VALL:
            RUNS.append((g, g + 1, 1 if g in V1 else 2))
            g += 1
        else:
            e = g
            while e < NGRP and e not in VALL:
                e += 1
            RUNS.append((g, e, 0))
            g = e
    order, c = [], 0
    for fc in CHUNKS:
        order += [c + t for t in range(0, fc, 128)]
        order += [TC + c + t for t in range(0, fc, 128)]
        c += fc
    jobs = [(f, v) for f in order for v in range(len(V2))]
    mid = len(jobs) // 2
    EXTRA_JOBS = jobs[mid:mid + 6]
    jobs = jobs[:mid] + jobs[mid + 6:]
    nslots = (M // G) * (D // GR) - 6
    SLOT_JOBS = {}
    for j, job in enumerate(jobs):
        SLOT_JOBS.setdefault(j * nslots // len(jobs), []).append(job)

    def kernel(xT_hbm, wg_hbm, wu_hbm, wdT_hbm, oT_hbm,
               xT_v, x_v, wgs, wus, wds, wge, wue, wde, wgm, wum, wdm,
               acc, o_v, wT, gu, xtab, r_v, flag, sem):
        w_hbm = (wg_hbm, wu_hbm, wdT_hbm)
        w_small = (wgs, wus, wds)
        w_ext = (wge, wue, wde)
        w_main = (wgm, wum, wdm)
        flag[0] = 0
        krem = pl.ds(KM, KR)

        def ext_copy(k, j, s):
            return pltpu.make_async_copy(
                w_hbm[k].at[:, pl.ds(A + j * 128, 128)], w_ext[k].at[j],
                sem.at[s])

        def main_copy(k, p, s, r0=0, nr=D):
            return pltpu.make_async_copy(
                w_hbm[k].at[pl.ds(r0, nr), pl.ds(A + NE * 128 + p * TC, TC)],
                w_main[k].at[p, pl.ds(r0, nr), :], sem.at[s])

        def x_slab_copy(k, q0, nq, s):
            idx = (pl.ds(*SLAB[k]), pl.ds(q0 * Q, nq * Q))
            return pltpu.make_async_copy(
                xT_hbm.at[idx], xT_v.at[idx], sem.at[s])

        def w_slab_copies(k, s):
            return [pltpu.make_async_copy(
                w_hbm[m].at[pl.ds(*SLAB[k]), pl.ds(0, A)],
                w_small[m].at[pl.ds(*SLAB[k]), :], sem.at[s])
                for m in range(2)]

        def out_copy(c0, d0, nd):
            return pltpu.make_async_copy(
                o_v.at[pl.ds(d0, nd), pl.ds(c0, G)],
                oT_hbm.at[pl.ds(d0, nd), pl.ds(c0, G)], sem.at[2])

        def start(group):
            for cp in group:
                cp.start()

        def wait(group):
            for cp in group:
                cp.wait()

        g_w0 = w_slab_copies(0, 0)
        g_stage = []
        for si, (slabs, parts) in enumerate(STAGES):
            grp = []
            for k, q0, nq in parts:
                if k in slabs:
                    grp += w_slab_copies(k, si + 1)
                grp.append(x_slab_copy(k, q0, nq, si + 1))
            g_stage.append(grp)
        g_last = ([x_slab_copy(k, q0, nq, 3) for k, q0, nq in LEFT]
                  + w_slab_copies(3, 3)
                  + [x_slab_copy(3, 0, 4, 3),
                     pltpu.make_async_copy(
                         wdT_hbm.at[:, pl.ds(0, A)], wds, sem.at[3])]
                  + [main_copy(k, 0, 3, KM, KR) for k in range(2)])
        g_main0 = ([main_copy(k, 0, 0, 0, KM) for k in range(2)]
                   + [main_copy(2, 0, 0)]
                   + [ext_copy(k, 0, 0) for k in range(3)]
                   + [main_copy(k, 1, 0) for k in range(2)])
        g_rest = ([main_copy(2, 1, 1)]
                  + [main_copy(k, p, 1)
                     for p in range(2, NP) for k in range(3)]
                  + [ext_copy(k, j, 1) for j in range(1, NE) for k in range(3)])

        start(g_w0 + [cp for grp in g_stage for cp in grp] + g_last)

        def transpose_w(k):
            ks = pl.ds(*SLAB[k])
            wT[pl.ds(0, A), ks] = wgs[ks, :].T
            wT[pl.ds(A, A), ks] = wus[ks, :].T

        def gate_up_t(k, q):
            ks = pl.ds(*SLAB[k])
            return _mm(wT[:, ks], xT_v[ks, pl.ds(q * Q, Q)])

        def accumulate(parts):
            for k, q0, nq in parts:
                for q in range(q0, q0 + nq):
                    if k == 0:
                        gu[q] = gate_up_t(k, q)
                    else:
                        gu[q] = gu[q] + gate_up_t(k, q)

        def warmup():
            wait(g_w0)
            start(g_main0)
            transpose_w(0)
            for si, (slabs, parts) in enumerate(STAGES):
                wait(g_stage[si])
                if si == 0:
                    start(g_rest)
                for k in slabs:
                    transpose_w(k)
                accumulate(parts)
            wait(g_last)
            transpose_w(3)
            accumulate(LEFT)
            for vi, grp in enumerate(VALL):
                t0 = (grp * GR // 128) * 128
                xt = xT_v[krem, pl.ds(t0, 128)].astype(_F32).T
                xg = xt[grp * GR - t0:grp * GR - t0 + GR]
                for k in range(KR):
                    xtab[k, pl.ds(vi * GR, GR), :] = jnp.broadcast_to(
                        xg[:, k:k + 1], (GR, 128))
            h_t = []
            for q in range(4):
                v = gu[q] + gate_up_t(3, q)
                h_t.append(_act2(v[:A], v[A:]).astype(_BF16))
            for q in range(4):
                qs = pl.ds((q % 2) * Q, Q)
                acc[q // 2, :, qs] = _mm(wds[...], h_t[q])
                x_v[q // 2, qs, :] = xT_v[:, pl.ds(q * Q, Q)].T
            xr2 = jnp.concatenate(
                [x_v[grp * GR // H, pl.ds(grp * GR % H, GR), krem]
                 for grp in V2], axis=0)
            for r0 in (0, NV2 // 2):
                rs = pl.ds(r0, NV2 // 2)
                xh = xr2[r0:r0 + NV2 // 2]
                r_v[rs, pl.ds(0, TC)] = _mm(xh, wgm[0, krem, :])
                r_v[rs, pl.ds(TC, TC)] = _mm(xh, wum[0, krem, :])
            wait(g_main0)

        def rows_bcast(w, f):
            return [jnp.broadcast_to(w[k:k + 1, f:f + 128], (GR, 128))
                    for k in range(KR)]

        def body(i, carry):
            pl.when(i == 0)(warmup)

            @pl.when(i == 1)
            def _():
                wait(g_rest)

            never = flag[0] != 0
            xm = x_v[:, :, pl.ds(0, KM)].reshape(M, KM)
            xr_all = x_v[:, :, krem].reshape(M, KR)
            xrem = jnp.concatenate(
                [xr_all[a * GR:b * GR] for a, b, v in RUNS if v == 0], axis=0)
            nxt = jnp.minimum(i + 1, NP - 1)
            w_next = jnp.concatenate(
                [wgm[nxt, krem, :], wum[nxt, krem, :]], axis=1).astype(_F32)
            w_next_b = {}

            def run_job(job, after):
                f, v = job
                if f not in w_next_b:
                    w_next_b[f] = rows_bcast(w_next, f)
                s = None
                for k in range(KR):
                    p = (xtab[k, pl.ds((len(V1) + v) * GR, GR), :]
                         * w_next_b[f][k])
                    s = jnp.where(never, after, p) if s is None else s + p
                r_v[pl.ds(v * GR, GR), pl.ds(f, 128)] = s

            h_chunks, c = [], 0
            for fc in CHUNKS:
                cs = pl.ds(c, fc)
                w_km = jnp.concatenate(
                    [wgm[i, pl.ds(0, KM), cs], wum[i, pl.ds(0, KM), cs]],
                    axis=1)
                w_kr = jnp.concatenate(
                    [wgm[i, krem, cs], wum[i, krem, cs]], axis=1)
                main = _mm(xm, w_km)
                if fc % 256 == 0:
                    rem = _mm(xrem, w_kr)
                else:
                    hv = (MV // 32) * 16
                    rem = jnp.concatenate(
                        [_mm(xrem[:hv], w_kr), _mm(xrem[hv:], w_kr)], axis=0)
                w_f = w_kr.astype(_F32)
                w_b = [rows_bcast(w_f, f) for f in range(0, 2 * fc, 128)]
                pieces, mi = [], 0
                for a, b, v in RUNS:
                    part = main[a * GR:b * GR]
                    if v == 0:
                        n = (b - a) * GR
                        pieces.append(part + rem[mi:mi + n])
                        mi += n
                    elif v == 2:
                        rs = pl.ds(V2.index(a) * GR, GR)
                        pieces.append(part + jnp.concatenate(
                            [r_v[rs, cs], r_v[rs, pl.ds(TC + c, fc)]], axis=1))
                    else:
                        rs = pl.ds(V1.index(a) * GR, GR)
                        tiles = []
                        for f in range(0, 2 * fc, 128):
                            s = None
                            for k in range(KR):
                                p = xtab[k, rs, :] * w_b[f // 128][k]
                                s = p if s is None else s + p
                            tiles.append(s + part[:, f:f + 128])
                        pieces.append(jnp.concatenate(tiles, axis=1))
                g_u = jnp.concatenate(pieces, axis=0)
                h_chunks.append(_act2(g_u[:, :fc], g_u[:, fc:]))
                c += fc
            hf = jnp.concatenate(h_chunks, axis=1)

            wd = wdm[i]
            for g in range(M // G):
                if g == H // G:
                    hh = i & 1
                    et = lax.shift_right_logical(i, 1)
                    he = []
                    for r in range(2):
                        xe = x_v[hh, pl.ds(r * Q, Q), :]
                        ge = _mm(xe, wge[et])
                        for j, job in enumerate(EXTRA_JOBS[3 * r:3 * r + 3]):
                            pg = j * (Q // GR) // 3
                            run_job(job, ge[pg * GR:(pg + 1) * GR])
                        he.append(_act2(ge, _mm(xe, wue[et])).astype(_BF16))
                    acc[hh] += _mm_nt(wde[et], jnp.concatenate(he, axis=0))
                c0 = g * G
                hq, cc = divmod(c0, H)
                osl = pl.ds(cc, G)
                val = acc[hq, :, osl] + _mm_nt(
                    wd, hf[c0:c0 + G].astype(_BF16))
                for rb in range(D // GR):
                    for job in SLOT_JOBS.get(g * (D // GR) + rb, []):
                        run_job(job, val[rb * GR:(rb + 1) * GR])
                acc[hq, :, osl] = val
                d0 = 0
                for nd in (LAST if c0 + G == M else (D,)):
                    o_v[pl.ds(d0, nd), pl.ds(c0, G)] = (
                        val[d0:d0 + nd] * 0.5).astype(o_v.dtype)

                    @pl.when(i == NP - 1)
                    def _():
                        out_copy(c0, d0, nd).start()

                    d0 += nd
            return carry

        lax.fori_loop(0, NP, body, 0)
        pltpu.make_async_copy(o_v, o_v, sem.at[2]).wait()

    any_spec = pl.BlockSpec(memory_space=pl.ANY)
    out_t = pl.pallas_call(
        kernel,
        in_specs=[any_spec] * 4,
        out_specs=any_spec,
        out_shape=jax.ShapeDtypeStruct((D, M), x.dtype),
        scratch_shapes=[
            pltpu.VMEM((D, M), _BF16),
            pltpu.VMEM((2, H, D), _BF16),
            pltpu.VMEM((D, A), _BF16),
            pltpu.VMEM((D, A), _BF16),
            pltpu.VMEM((D, A), _BF16),
            pltpu.VMEM((NE, D, 128), _BF16),
            pltpu.VMEM((NE, D, 128), _BF16),
            pltpu.VMEM((NE, D, 128), _BF16),
            pltpu.VMEM((NP, D, TC), _BF16),
            pltpu.VMEM((NP, D, TC), _BF16),
            pltpu.VMEM((NP, D, TC), _BF16),
            pltpu.VMEM((2, D, H), _F32),
            pltpu.VMEM((D, M), _BF16),
            pltpu.VMEM((2 * A, D), _BF16),
            pltpu.VMEM((4, 2 * A, Q), _F32),
            pltpu.VMEM((KR, NV + 8, 128), _F32),
            pltpu.VMEM((NV2, 2 * TC), _F32),
            pltpu.SMEM((1,), jnp.int32),
            pltpu.SemaphoreType.DMA((4,)),
        ],
        compiler_params=pltpu.CompilerParams(
            vmem_limit_bytes=110 * 1024 * 1024),
    )(x.reshape(M, D).T, w_gate, w_up, w_down.T)
    return out_t.T.reshape(B, S, D)
```

```python
import math

import jax
import jax.numpy as jnp
from jax import lax
import jax.experimental.pallas as pl
import jax.experimental.pallas.tpu as pltpu

_NT = (((1,), (1,)), ((), ()))
_F32 = jnp.float32
_BF16 = jnp.bfloat16
_C1 = math.sqrt(2.0 / math.pi)
_C2 = _C1 * 0.044715


def _act2(g, u):
    t = jnp.tanh(g * (_C1 + _C2 * (g * g)))
    return (g * (1.0 + t)) * u


def _mm(a, b):
    return jnp.dot(a, b, preferred_element_type=_F32)


def _mm_nt(a, b):
    return lax.dot_general(a, b, _NT, preferred_element_type=_F32)


@jax.jit
def pallas_standalone__geglu_ffn__prompt_kernel(
    x: jax.Array,
    w_gate: jax.Array,
    w_up: jax.Array,
    w_down: jax.Array,
):
    B, S, D = x.shape
    F = w_gate.shape[1]
    M = B * S
    assert (M, D, F) == (2048, 576, 4608)

    A = 384
    NE = 3
    TC = 640
    NP = 6
    CHUNKS = (256, 256, 128)
    Q, H = 512, 1024
    G = 128
    LAST = (288, 144, 96, 32, 16)
    KM, KR = 512, 64
    assert A + NE * 128 + NP * TC == F and sum(CHUNKS) == TC
    assert sum(LAST) == D and KM + KR == D and 2 * NE == NP

    SLAB = ((512, 64), (0, 128), (128, 128), (256, 256))
    STAGES = (
        ((), ((0, 0, 3),)),
        ((1, 2), ((0, 3, 1), (1, 0, 4), (2, 0, 1))),
    )
    LEFT = ((2, 1, 3),)

    GR = 16
    NGRP = M // GR
    V1 = [12 + 10 * j for j in range(12)]
    rest = [g for g in range(NGRP) if g not in V1]
    V2 = [rest[(2 * j + 1) * len(rest) // 16] for j in range(8)]
    VALL = V1 + V2
    NV, NV2 = GR * len(VALL), GR * len(V2)
    MV = M - NV
    assert len(VALL) % 5 == 0
    RUNS, g = [], 0
    while g < NGRP:
        if g in VALL:
            RUNS.append((g, g + 1, 1 if g in V1 else 2))
            g += 1
        else:
            e = g
            while e < NGRP and e not in VALL:
                e += 1
            RUNS.append((g, e, 0))
            g = e
    order, c = [], 0
    for fc in CHUNKS:
        order += [c + t for t in range(0, fc, 128)]
        order += [TC + c + t for t in range(0, fc, 128)]
        c += fc
    jobs = [(f, v) for f in order for v in range(len(V2))]
    mid = len(jobs) // 2
    EXTRA_JOBS = jobs[mid:mid + 6]
    jobs = jobs[:mid] + jobs[mid + 6:]
    nslots = (M // G) * (D // GR) - 6
    SLOT_JOBS = {}
    for j, job in enumerate(jobs):
        SLOT_JOBS.setdefault(j * nslots // len(jobs), []).append(job)

    def kernel(xT_hbm, wg_hbm, wu_hbm, wdT_hbm, oT_hbm,
               xT_v, x_v, wgs, wus, wds, wge, wue, wde, wgm, wum, wdm,
               acc, o_v, wT, gu, xtab, r_v, flag, sem):
        w_hbm = (wg_hbm, wu_hbm, wdT_hbm)
        w_small = (wgs, wus, wds)
        w_ext = (wge, wue, wde)
        w_main = (wgm, wum, wdm)
        flag[0] = 0
        krem = pl.ds(KM, KR)

        def ext_copy(k, j, s):
            return pltpu.make_async_copy(
                w_hbm[k].at[:, pl.ds(A + j * 128, 128)], w_ext[k].at[j],
                sem.at[s])

        def main_copy(k, p, s, r0=0, nr=D):
            return pltpu.make_async_copy(
                w_hbm[k].at[pl.ds(r0, nr), pl.ds(A + NE * 128 + p * TC, TC)],
                w_main[k].at[p, pl.ds(r0, nr), :], sem.at[s])

        def x_slab_copy(k, q0, nq, s):
            idx = (pl.ds(*SLAB[k]), pl.ds(q0 * Q, nq * Q))
            return pltpu.make_async_copy(
                xT_hbm.at[idx], xT_v.at[idx], sem.at[s])

        def w_slab_copies(k, s):
            return [pltpu.make_async_copy(
                w_hbm[m].at[pl.ds(*SLAB[k]), pl.ds(0, A)],
                w_small[m].at[pl.ds(*SLAB[k]), :], sem.at[s])
                for m in range(2)]

        def out_copy(c0, d0, nd):
            return pltpu.make_async_copy(
                o_v.at[pl.ds(d0, nd), pl.ds(c0, G)],
                oT_hbm.at[pl.ds(d0, nd), pl.ds(c0, G)], sem.at[2])

        def start(group):
            for cp in group:
                cp.start()

        def wait(group):
            for cp in group:
                cp.wait()

        g_w0 = w_slab_copies(0, 0)
        g_stage = []
        for si, (slabs, parts) in enumerate(STAGES):
            grp = []
            for k, q0, nq in parts:
                if k in slabs:
                    grp += w_slab_copies(k, si + 1)
                grp.append(x_slab_copy(k, q0, nq, si + 1))
            g_stage.append(grp)
        g_last = ([x_slab_copy(k, q0, nq, 3) for k, q0, nq in LEFT]
                  + w_slab_copies(3, 3)
                  + [x_slab_copy(3, 0, 4, 3),
                     pltpu.make_async_copy(
                         wdT_hbm.at[:, pl.ds(0, A)], wds, sem.at[3])]
                  + [main_copy(k, 0, 3, KM, KR) for k in range(2)])
        g_main0 = ([main_copy(k, 0, 0, 0, KM) for k in range(2)]
                   + [main_copy(2, 0, 0)]
                   + [ext_copy(k, 0, 0) for k in range(3)]
                   + [main_copy(k, 1, 0) for k in range(2)])
        g_rest = ([main_copy(2, 1, 1)]
                  + [main_copy(k, p, 1)
                     for p in range(2, NP) for k in range(3)]
                  + [ext_copy(k, j, 1) for j in range(1, NE) for k in range(3)])

        start(g_w0 + [cp for grp in g_stage for cp in grp] + g_last)

        def transpose_w(k):
            ks = pl.ds(*SLAB[k])
            wT[pl.ds(0, A), ks] = wgs[ks, :].T
            wT[pl.ds(A, A), ks] = wus[ks, :].T

        def gate_up_t(k, q):
            ks = pl.ds(*SLAB[k])
            return _mm(wT[:, ks], xT_v[ks, pl.ds(q * Q, Q)])

        def accumulate(parts):
            for k, q0, nq in parts:
                for q in range(q0, q0 + nq):
                    if k == 0:
                        gu[q] = gate_up_t(k, q)
                    else:
                        gu[q] = gu[q] + gate_up_t(k, q)

        def warmup():
            wait(g_w0)
            start(g_main0)
            transpose_w(0)
            for si, (slabs, parts) in enumerate(STAGES):
                wait(g_stage[si])
                if si == 0:
                    start(g_rest)
                for k in slabs:
                    transpose_w(k)
                accumulate(parts)
            wait(g_last)
            transpose_w(3)
            accumulate(LEFT)
            xgs = []
            for grp in VALL:
                t0 = (grp * GR // 128) * 128
                xt = xT_v[krem, pl.ds(t0, 128)].astype(_F32).T
                xgs.append(xt[grp * GR - t0:grp * GR - t0 + GR])
            for v0 in range(0, len(VALL), 5):
                xg = jnp.concatenate(xgs[v0:v0 + 5], axis=0)
                for k in range(KR):
                    xtab[k, pl.ds(v0 * GR, 5 * GR), :] = jnp.broadcast_to(
                        xg[:, k:k + 1], (5 * GR, 128))
            h_t = []
            for q in range(4):
                v = gu[q] + gate_up_t(3, q)
                h_t.append(_act2(v[:A], v[A:]).astype(_BF16))
            for q in range(4):
                qs = pl.ds((q % 2) * Q, Q)
                acc[q // 2, :, qs] = _mm(wds[...], h_t[q])
                x_v[q // 2, qs, :] = xT_v[:, pl.ds(q * Q, Q)].T
            xr2 = jnp.concatenate(
                [x_v[grp * GR // H, pl.ds(grp * GR % H, GR), krem]
                 for grp in V2], axis=0)
            for r0 in (0, NV2 // 2):
                rs = pl.ds(r0, NV2 // 2)
                xh = xr2[r0:r0 + NV2 // 2]
                r_v[rs, pl.ds(0, TC)] = _mm(xh, wgm[0, krem, :])
                r_v[rs, pl.ds(TC, TC)] = _mm(xh, wum[0, krem, :])
            wait(g_main0)

        def rows_bcast(w):
            return jnp.stack(
                [jnp.broadcast_to(w[k:k + 1], (GR, w.shape[1]))
                 for k in range(KR)], axis=0)

        def body(i, carry):
            pl.when(i == 0)(warmup)

            @pl.when(i == 1)
            def _():
                wait(g_rest)

            never = flag[0] != 0
            xm = x_v[:, :, pl.ds(0, KM)].reshape(M, KM)
            xr_all = x_v[:, :, krem].reshape(M, KR)
            xrem = jnp.concatenate(
                [xr_all[a * GR:b * GR] for a, b, v in RUNS if v == 0], axis=0)
            nxt = jnp.minimum(i + 1, NP - 1)
            w_next = jnp.concatenate(
                [wgm[nxt, krem, :], wum[nxt, krem, :]], axis=1).astype(_F32)
            w_next_b = []

            def run_job(job, after):
                f, v = job
                if not w_next_b:
                    w_next_b.append(rows_bcast(w_next))
                w_t = w_next_b[0][:, :, f:f + 128]
                rs = pl.ds((len(V1) + v) * GR, GR)
                s = None
                for k0 in range(0, KR, 8):
                    p = xtab[pl.ds(k0, 8), rs, :] * w_t[k0:k0 + 8]
                    if s is None:
                        p = jnp.concatenate(
                            [jnp.where(never, after, p[0])[None], p[1:]],
                            axis=0)
                    else:
                        p = jnp.concatenate([s[None], p], axis=0)
                    s = jnp.sum(p, axis=0)
                r_v[pl.ds(v * GR, GR), pl.ds(f, 128)] = s

            h_chunks, c = [], 0
            for fc in CHUNKS:
                cs = pl.ds(c, fc)
                w_km = jnp.concatenate(
                    [wgm[i, pl.ds(0, KM), cs], wum[i, pl.ds(0, KM), cs]],
                    axis=1)
                w_kr = jnp.concatenate(
                    [wgm[i, krem, cs], wum[i, krem, cs]], axis=1)
                main = _mm(xm, w_km)
                if fc % 256 == 0:
                    rem = _mm(xrem, w_kr)
                else:
                    hv = (MV // 32) * 16
                    rem = jnp.concatenate(
                        [_mm(xrem[:hv], w_kr), _mm(xrem[hv:], w_kr)], axis=0)
                w_b = rows_bcast(w_kr.astype(_F32))
                w_b = [w_b[:, :, f:f + 128] for f in range(0, 2 * fc, 128)]
                pieces, mi = [], 0
                for a, b, v in RUNS:
                    part = main[a * GR:b * GR]
                    if v == 0:
                        n = (b - a) * GR
                        pieces.append(part + rem[mi:mi + n])
                        mi += n
                    elif v == 2:
                        rs = pl.ds(V2.index(a) * GR, GR)
                        pieces.append(part + jnp.concatenate(
                            [r_v[rs, cs], r_v[rs, pl.ds(TC + c, fc)]], axis=1))
                    else:
                        rs = pl.ds(V1.index(a) * GR, GR)
                        tiles = [
                            jnp.sum(xtab[:, rs, :] * w_b[f // 128], axis=0)
                            + part[:, f:f + 128]
                            for f in range(0, 2 * fc, 128)]
                        pieces.append(jnp.concatenate(tiles, axis=1))
                g_u = jnp.concatenate(pieces, axis=0)
                h_chunks.append(_act2(g_u[:, :fc], g_u[:, fc:]))
                c += fc
            hf = jnp.concatenate(h_chunks, axis=1)

            wd = wdm[i]
            for g in range(M // G):
                if g == H // G:
                    hh = i & 1
                    et = lax.shift_right_logical(i, 1)
                    he = []
                    for r in range(2):
                        xe = x_v[hh, pl.ds(r * Q, Q), :]
                        ge = _mm(xe, wge[et])
                        for j, job in enumerate(EXTRA_JOBS[3 * r:3 * r + 3]):
                            pg = j * (Q // GR) // 3
                            run_job(job, ge[pg * GR:(pg + 1) * GR])
                        he.append(_act2(ge, _mm(xe, wue[et])).astype(_BF16))
                    acc[hh] += _mm_nt(wde[et], jnp.concatenate(he, axis=0))
                c0 = g * G
                hq, cc = divmod(c0, H)
                osl = pl.ds(cc, G)
                val = acc[hq, :, osl] + _mm_nt(
                    wd, hf[c0:c0 + G].astype(_BF16))
                for rb in range(D // GR):
                    for job in SLOT_JOBS.get(g * (D // GR) + rb, []):
                        run_job(job, val[rb * GR:(rb + 1) * GR])
                acc[hq, :, osl] = val
                d0 = 0
                for nd in (LAST if c0 + G == M else (D,)):
                    o_v[pl.ds(d0, nd), pl.ds(c0, G)] = (
                        val[d0:d0 + nd] * 0.5).astype(o_v.dtype)

                    @pl.when(i == NP - 1)
                    def _():
                        out_copy(c0, d0, nd).start()

                    d0 += nd
            return carry

        lax.fori_loop(0, NP, body, 0)
        pltpu.make_async_copy(o_v, o_v, sem.at[2]).wait()

    any_spec = pl.BlockSpec(memory_space=pl.ANY)
    out_t = pl.pallas_call(
        kernel,
        in_specs=[any_spec] * 4,
        out_specs=any_spec,
        out_shape=jax.ShapeDtypeStruct((D, M), x.dtype),
        scratch_shapes=[
            pltpu.VMEM((D, M), _BF16),
            pltpu.VMEM((2, H, D), _BF16),
            pltpu.VMEM((D, A), _BF16),
            pltpu.VMEM((D, A), _BF16),
            pltpu.VMEM((D, A), _BF16),
            pltpu.VMEM((NE, D, 128), _BF16),
            pltpu.VMEM((NE, D, 128), _BF16),
            pltpu.VMEM((NE, D, 128), _BF16),
            pltpu.VMEM((NP, D, TC), _BF16),
            pltpu.VMEM((NP, D, TC), _BF16),
            pltpu.VMEM((NP, D, TC), _BF16),
            pltpu.VMEM((2, D, H), _F32),
            pltpu.VMEM((D, M), _BF16),
            pltpu.VMEM((2 * A, D), _BF16),
            pltpu.VMEM((4, 2 * A, Q), _F32),
            pltpu.VMEM((KR, NV + 8, 128), _F32),
            pltpu.VMEM((NV2, 2 * TC), _F32),
            pltpu.SMEM((1,), jnp.int32),
            pltpu.SemaphoreType.DMA((4,)),
        ],
        compiler_params=pltpu.CompilerParams(
            vmem_limit_bytes=110 * 1024 * 1024),
    )(x.reshape(M, D).T, w_gate, w_up, w_down.T)
    return out_t.T.reshape(B, S, D)
```
